```python
import jax
import jax.numpy as jnp

def _softmax(x, axis=-1):
    return jax.nn.softmax(x, axis=axis)
def _gelu(x):
    return jax.nn.gelu(x, approximate=True)
def _silu(x):
    return jax.nn.silu(x)
def _sigmoid(x):
    return jax.nn.sigmoid(x)
def _layernorm(x, axis=-1, eps=1e-5):
    m = jnp.mean(x, axis=axis, keepdims=True)
    v = jnp.var(x, axis=axis, keepdims=True)
    return (x - m) / jnp.sqrt(v + eps)
def _scatter_add(tgt, idx, src, axis=0):
    return tgt.at[idx].add(src)
def _segment_sum(src, seg, n):
    return jax.ops.segment_sum(src, seg, n)
class _Rng:
    def __init__(self, key):
        self._k = key
    def _next(self):
        self._k, sub = jax.random.split(self._k)
        return sub
    def normal(self, shape):
        return jax.random.normal(self._next(), shape, dtype=jnp.bfloat16)
    def randint(self, lo, hi, shape):
        return jax.random.randint(self._next(), shape, lo, hi, dtype=jnp.int32)
    def uniform(self, shape, lo=0.0, hi=1.0):
        return jax.random.uniform(self._next(), shape, jnp.bfloat16, lo, hi)
    def permutation(self, n):
        return jax.random.permutation(self._next(), n)


kernel_name = 'standalone__standard_2d_1d_3d_conv__vision'

def setup_inputs():
    _rng = _Rng(jax.random.key(int.from_bytes(__import__("os").urandom(4), "little")))
    _w = (lambda a: (lambda t: t.astype(jnp.bfloat16) if jnp.issubdtype(t.dtype, jnp.floating) else t)(jnp.asarray(a)))
    H = W = 384
    C = 384
    K = 1
    return {
        "x": _w((lambda *s: _rng.normal(s) * 0.05)(1, H, W, C)),
        "w": _w((lambda *s: _rng.normal(s) * 0.05)(K, K, C, C)),
        "b": _w((lambda *s: _rng.normal(s) * 0.05)(C)),
    }

def reference(x, w, b):
    B, H, W, Cin = x.shape
    K = w.shape[0]
    pl = (K - 1) // 2
    pr = K // 2
    xp = jnp.pad(x, ((0, 0), (pl, pr), (pl, pr), (0, 0)))
    out = sum(
        jnp.einsum('bhwc,cd->bhwd', xp[:, i:i+H, j:j+W, :], w[i, j])
        for i in range(K) for j in range(K)
    )
    return out + b[None, None, None, :]
```

```python
import jax
import jax.numpy as jnp
from jax import lax
import jax.experimental.pallas as pl
import jax.experimental.pallas.tpu as pltpu

NSTREAM = 6
CHUNK = 384
WPIECE = 48
RCHUNKS = 2
SWITCH = 38
W_FIRST = 32
W_STEP = 14


@jax.jit
def pallas_standalone__standard_2d_1d_3d_conv__vision_kernel(
    x: jax.Array,
    w: jax.Array,
    b: jax.Array,
):
    B, H, W, Cin = x.shape
    Cout = w.shape[-1]
    assert w.shape[:2] == (1, 1) and Cin == Cout
    M = B * H * W
    K, G, T, RG = NSTREAM, CHUNK, WPIECE, RCHUNKS
    S = M // K
    n_steps = S // G
    n_writes = S // T
    n_reads = n_steps // RG
    w_per_step = G // T
    assert K * S == M and n_steps * G == S and n_reads * RG == n_steps
    assert w_per_step * T == G and SWITCH % RG == 0
    assert W_FIRST <= SWITCH * w_per_step
    for s in range(SWITCH, n_steps):
        assert W_FIRST + (s - SWITCH + 1) * W_STEP <= (s + 1) * w_per_step
    w_issued = W_FIRST + (n_steps - SWITCH) * W_STEP
    assert w_issued <= n_writes

    def kernel(x_hbm, w_hbm, b_hbm, o_hbm, buf, w_v, b_v, rsem, psem, wsem):
        def read(r):
            rows = pl.ds(pl.multiple_of(r * (RG * G), 16), RG * G)
            return pltpu.make_async_copy(
                x_hbm.at[:, rows, :], buf.at[:, rows, :], rsem.at[r])

        def start_writes(lo, n):
            def body(i, c):
                rows = pl.ds(pl.multiple_of((lo + i) * T, 16), T)
                pltpu.make_async_copy(
                    buf.at[:, rows, :], o_hbm.at[:, rows, :], wsem).start()
                return c
            lax.fori_loop(0, n, body, 0)

        def start_read(r, c):
            read(r).start()
            return c

        def wait_read(r, c):
            read(r).wait()
            return c

        copy_w = pltpu.make_async_copy(w_hbm, w_v, psem.at[0])
        copy_b = pltpu.make_async_copy(b_hbm, b_v, psem.at[1])
        lax.fori_loop(0, 1, start_read, 0)
        copy_w.start()
        copy_b.start()
        lax.fori_loop(1, n_reads, start_read, 0)
        copy_w.wait()
        copy_b.wait()

        def step(g, c):
            @pl.when(jnp.logical_and(g < SWITCH, g % RG == 0))
            def _():
                read(g // RG).wait()

            @pl.when(g == SWITCH)
            def _():
                lax.fori_loop(SWITCH // RG, n_reads, wait_read, 0)
                start_writes(0, W_FIRST)

            rows = pl.ds(pl.multiple_of(g * G, 16), G)
            xs = buf[:, rows, :].reshape(K * G, Cin)
            acc = jnp.dot(xs, w_v[0, 0], preferred_element_type=jnp.float32)
            y = acc + b_v[...].astype(jnp.float32)[None, :]
            buf[:, rows, :] = y.astype(buf.dtype).reshape(K, G, Cout)

            @pl.when(g >= SWITCH)
            def _():
                start_writes(W_FIRST + (g - SWITCH) * W_STEP, W_STEP)

            return c

        lax.fori_loop(0, n_steps, step, 0)
        start_writes(w_issued, n_writes - w_issued)
        pltpu.make_async_copy(buf, o_hbm, wsem).wait()

    out = pl.pallas_call(
        kernel,
        in_specs=[pl.BlockSpec(memory_space=pl.ANY)] * 3,
        out_specs=pl.BlockSpec(memory_space=pl.ANY),
        out_shape=jax.ShapeDtypeStruct((K, S, Cout), x.dtype),
        scratch_shapes=[
            pltpu.VMEM((K, S, Cin), x.dtype),
            pltpu.VMEM(w.shape, w.dtype),
            pltpu.VMEM(b.shape, b.dtype),
            pltpu.SemaphoreType.DMA((n_reads,)),
            pltpu.SemaphoreType.DMA((2,)),
            pltpu.SemaphoreType.DMA(()),
        ],
        compiler_params=pltpu.CompilerParams(
            vmem_limit_bytes=122 * 1024 * 1024,
        ),
    )(x.reshape(K, S, Cin), w, b)
    return out.reshape(B, H, W, Cout)
```

```python
import jax
import jax.numpy as jnp
from jax import lax
import jax.experimental.pallas as pl
import jax.experimental.pallas.tpu as pltpu

NSTREAM = 6
CHUNK = 384
UNIT = 48
SUB = 128
PIECE = 32
SWITCH = 38
LEAD = 4
L_STEP = 11
W_FIRST = 16
W_STEP = 14
EARLY = 2


def _spread(n, m):
    return [s for s in range(m) if (s * n) // m != ((s + 1) * n) // m]


@jax.jit
def pallas_standalone__standard_2d_1d_3d_conv__vision_kernel(
    x: jax.Array,
    w: jax.Array,
    b: jax.Array,
):
    B, H, W, C = x.shape
    assert w.shape == (1, 1, C, C) and b.shape == (C,)
    K, G, T, P = NSTREAM, CHUNK, UNIT, PIECE
    S = B * H * W // K
    n_steps = S // G
    n_pairs = n_steps // 2
    upc = G // T
    n_units = n_pairs * upc
    spr = G // SUB
    n_sub = K * spr
    assert K * S == B * H * W and 2 * n_pairs * G == S
    assert upc * T == G and spr * SUB == G and G % P == 0

    h_rows = [(SWITCH // 2) * spr * P, ((SWITCH + 1) // 2) * spr * P]
    n_low = [n_units - r // T for r in h_rows]
    lead = [(LEAD + 1) // 2 * upc, LEAD // 2 * upc]
    assert all(r % T == 0 and (n * T) % P == 0 for r, n in zip(h_rows, n_low))
    order = [(c % 2, c // 2 * upc + i) for c in range(LEAD) for i in range(upc)]
    for g in range(SWITCH):
        assert all((g % 2, g // 2 * upc + i) in order for i in range(upc))
        p = 1 - g % 2
        lo = lead[p] + g // 2 * L_STEP
        order += [(p, u) for u in range(lo, min(lo + L_STEP, n_low[p]))]
    assert len(order) == sum(n_low)
    late = {}
    for p, u in order[len(order) - EARLY:]:
        late[2 * (u // upc) + p] = late.get(2 * (u // upc) + p, 0) + 1
    assert min(late) >= SWITCH
    assert W_FIRST <= SWITCH * upc
    for g in range(SWITCH, n_steps):
        assert W_FIRST + (g - SWITCH + 1) * W_STEP <= g * upc
    w_in_loop = W_FIRST + (n_steps - SWITCH) * W_STEP
    assert w_in_loop <= 2 * n_units
    l_slots = _spread(L_STEP, n_sub)
    w_slots = _spread(W_STEP, n_sub)

    def kernel(x_hbm, w_hbm, b_hbm, o_hbm, buf_a, buf_b, w_v, b_v,
               lsem, hsem, psem, wsem):
        def in_slots(par, j, n=None):
            ref, j = (buf_a, j) if par == 0 else (buf_b, j + 1)
            return ref.at[j] if n is None else ref.at[pl.ds(j, n)]

        def out_slot(par, j):
            return buf_b.at[j] if par == 0 else buf_a.at[j]

        def locate(par, row):
            j = lax.div(row, G)
            off = pl.multiple_of(lax.rem(row, G), 16)
            return j, off, pl.multiple_of((2 * j + par) * G + off, 16)

        def start_low(par, u):
            j, off, row = locate(par, u * T)
            pltpu.make_async_copy(
                x_hbm.at[:, pl.ds(row, T), :],
                in_slots(par, j).at[:, pl.ds(off, T), :],
                lsem.at[2 * j + par]).start(priority=1)

        def start_high(par, n, s):
            j, off, row = locate(par, n_low[par] * T + (n * spr + s % spr) * P)
            pltpu.make_async_copy(
                x_hbm.at[s // spr, pl.ds(row, P), :],
                in_slots(par, j).at[s // spr, pl.ds(off, P), :],
                hsem.at[par]).start(priority=0)

        def start_write(u, enable=True):
            c = lax.div(u, upc)
            off = pl.multiple_of(lax.rem(u, upc) * T, 16)
            row = pl.multiple_of(u * T, 16)
            for par in range(2):
                @pl.when(jnp.logical_and(lax.rem(c, 2) == par, enable))
                def _():
                    pltpu.make_async_copy(
                        out_slot(par, lax.div(c, 2)).at[:, pl.ds(off, T), :],
                        o_hbm.at[:, pl.ds(row, T), :], wsem).start()

        def start_writes(lo, hi):
            def body(u, carry):
                start_write(u)
                return carry
            lax.fori_loop(lo, hi, body, 0)

        def wait(view, sem):
            pltpu.make_async_copy(view, view, sem).wait()

        copy_w = pltpu.make_async_copy(w_hbm, w_v, psem.at[0])
        copy_b = pltpu.make_async_copy(b_hbm, b_v, psem.at[1])
        for c in range(LEAD):
            def lead_body(i, carry, c=c):
                start_low(c % 2, c // 2 * upc + i)
                return carry
            lax.fori_loop(0, upc, lead_body, 0)
            if c == 0:
                copy_w.start()
                copy_b.start()
        copy_w.wait()
        copy_b.wait()

        def switch():
            for par in range(2):
                j, r = divmod(n_low[par] * T, G)
                if r:
                    wait(in_slots(par, j).at[:, pl.ds(r, G - r), :], hsem.at[par])
                    j += 1
                wait(in_slots(par, j, n_pairs - j), hsem.at[par])
            held = []
            for c in range(SWITCH, n_steps):
                n = min(upc, n_low[c % 2] - c // 2 * upc)
                m = n - late.get(c, 0)
                slot = in_slots(c % 2, c // 2)
                if m > 0:
                    wait(slot.at[:, pl.ds(0, m * T), :], lsem.at[c])
                if n > max(m, 0):
                    held.append((slot.at[:, pl.ds(m * T, (n - m) * T), :], c))
            start_writes(0, W_FIRST)
            for view, c in held:
                wait(view, lsem.at[c])

        def step(par, j):
            g = 2 * j + par
            src = in_slots(par, j)
            dst = out_slot(par, j)

            @pl.when(g < SWITCH)
            def _():
                wait(src, lsem.at[g])

            if SWITCH % 2 == par:
                pl.when(g == SWITCH)(switch)

            bias = b_v[...].astype(jnp.float32)[None, :]
            for s in range(n_sub):
                k, r0 = s // spr, s % spr * SUB
                acc = jnp.dot(src[k, r0:r0 + SUB, :], w_v[0, 0],
                              preferred_element_type=jnp.float32)
                dst[k, r0:r0 + SUB, :] = (acc + bias).astype(dst.dtype)

                @pl.when(g < SWITCH)
                def _():
                    start_high(1 - par, j, s)

                if s in l_slots:
                    u = lead[1 - par] + j * L_STEP + l_slots.index(s)

                    @pl.when(u < n_low[1 - par])
                    def _():
                        start_low(1 - par, u)

                if s in w_slots:
                    u = W_FIRST + (g - SWITCH) * W_STEP + w_slots.index(s)
                    start_write(jnp.maximum(u, 0), g >= SWITCH)

        def pair(j, carry):
            step(0, j)
            step(1, j)
            return carry

        lax.fori_loop(0, n_pairs, pair, 0)
        start_writes(w_in_loop, 2 * n_units)
        wait(o_hbm, wsem)

    out = pl.pallas_call(
        kernel,
        in_specs=[pl.BlockSpec(memory_space=pl.ANY)] * 3,
        out_specs=pl.BlockSpec(memory_space=pl.ANY),
        out_shape=jax.ShapeDtypeStruct((K, S, C), x.dtype),
        scratch_shapes=[
            pltpu.VMEM((n_pairs, K, G, C), x.dtype),
            pltpu.VMEM((n_pairs + 1, K, G, C), x.dtype),
            pltpu.VMEM(w.shape, w.dtype),
            pltpu.VMEM(b.shape, b.dtype),
            pltpu.SemaphoreType.DMA((n_steps,)),
            pltpu.SemaphoreType.DMA((2,)),
            pltpu.SemaphoreType.DMA((2,)),
            pltpu.SemaphoreType.DMA(()),
        ],
        compiler_params=pltpu.CompilerParams(
            vmem_limit_bytes=124 * 1024 * 1024,
            disable_bounds_checks=True,
            disable_semaphore_checks=True,
        ),
    )(x.reshape(K, S, C), w, b)
    return out.reshape(B, H, W, C)
```

```python
import jax
import jax.numpy as jnp
from jax import lax
import jax.experimental.pallas as pl
import jax.experimental.pallas.tpu as pltpu

NSTREAM = 6
CHUNK = 384
UNIT = 48
SUB = 64
PIECE = 16
SWITCH = 38
LEAD = 3
L_STEP = 11
W_FIRST = 16
W_STEP = 14
EARLY = 2


def _spread(n, m):
    return [s for s in range(m) if (s * n) // m != ((s + 1) * n) // m]


@jax.jit
def pallas_standalone__standard_2d_1d_3d_conv__vision_kernel(
    x: jax.Array,
    w: jax.Array,
    b: jax.Array,
):
    B, H, W, C = x.shape
    assert w.shape == (1, 1, C, C) and b.shape == (C,)
    K, G, T, P = NSTREAM, CHUNK, UNIT, PIECE
    S = B * H * W // K
    n_steps = S // G
    n_pairs = n_steps // 2
    upc = G // T
    n_units = n_pairs * upc
    spr = G // SUB
    n_sub = K * spr
    assert K * S == B * H * W and 2 * n_pairs * G == S
    assert upc * T == G and spr * SUB == G and G % P == 0

    h_rows = [(SWITCH // 2) * spr * P, ((SWITCH + 1) // 2) * spr * P]
    n_low = [n_units - r // T for r in h_rows]
    lead = [(LEAD + 1) // 2 * upc, LEAD // 2 * upc]
    assert all(r % T == 0 and (n * T) % P == 0 for r, n in zip(h_rows, n_low))
    order = [(c % 2, c // 2 * upc + i) for c in range(LEAD) for i in range(upc)]
    for g in range(SWITCH):
        assert all((g % 2, g // 2 * upc + i) in order for i in range(upc))
        p = 1 - g % 2
        lo = lead[p] + g // 2 * L_STEP
        order += [(p, u) for u in range(lo, min(lo + L_STEP, n_low[p]))]
    rest = [(p, u) for p in range(2) for u in range(n_low[p])
            if (p, u) not in order]
    order += rest
    late = {}
    for p, u in order[len(order) - EARLY:]:
        late[2 * (u // upc) + p] = late.get(2 * (u // upc) + p, 0) + 1
    assert min(late) >= SWITCH
    assert W_FIRST <= SWITCH * upc
    for g in range(SWITCH, n_steps):
        assert W_FIRST + (g - SWITCH + 1) * W_STEP <= g * upc
    w_in_loop = W_FIRST + (n_steps - SWITCH) * W_STEP
    assert w_in_loop <= 2 * n_units
    l_slots = _spread(L_STEP, n_sub)
    w_slots = _spread(W_STEP, n_sub)

    def kernel(x_hbm, w_hbm, b_hbm, o_hbm, buf_a, buf_b, w_v, b_v,
               lsem, hsem, psem, wsem):
        def in_slots(par, j, n=None):
            ref, j = (buf_a, j) if par == 0 else (buf_b, j + 1)
            return ref.at[j] if n is None else ref.at[pl.ds(j, n)]

        def out_slot(par, j):
            return buf_b.at[j] if par == 0 else buf_a.at[j]

        def locate(par, row):
            j = lax.div(row, G)
            off = pl.multiple_of(lax.rem(row, G), 16)
            return j, off, pl.multiple_of((2 * j + par) * G + off, 16)

        def start_low(par, u):
            j, off, row = locate(par, u * T)
            pltpu.make_async_copy(
                x_hbm.at[:, pl.ds(row, T), :],
                in_slots(par, j).at[:, pl.ds(off, T), :],
                lsem.at[2 * j + par]).start(priority=1)

        def start_high(par, n, s):
            j, off, row = locate(par, n_low[par] * T + (n * spr + s % spr) * P)
            pltpu.make_async_copy(
                x_hbm.at[s // spr, pl.ds(row, P), :],
                in_slots(par, j).at[s // spr, pl.ds(off, P), :],
                hsem.at[par]).start(priority=0)

        def start_write(u, enable=True):
            c = lax.div(u, upc)
            off = pl.multiple_of(lax.rem(u, upc) * T, 16)
            row = pl.multiple_of(u * T, 16)
            for par in range(2):
                @pl.when(jnp.logical_and(lax.rem(c, 2) == par, enable))
                def _():
                    pltpu.make_async_copy(
                        out_slot(par, lax.div(c, 2)).at[:, pl.ds(off, T), :],
                        o_hbm.at[:, pl.ds(row, T), :], wsem).start()

        def start_writes(lo, hi):
            def body(u, carry):
                start_write(u)
                return carry
            lax.fori_loop(lo, hi, body, 0)

        def wait(view, sem):
            pltpu.make_async_copy(view, view, sem).wait()

        copy_w = pltpu.make_async_copy(w_hbm, w_v, psem.at[0])
        copy_b = pltpu.make_async_copy(b_hbm, b_v, psem.at[1])
        for c in range(LEAD):
            def lead_body(i, carry, c=c):
                start_low(c % 2, c // 2 * upc + i)
                return carry
            lax.fori_loop(0, upc, lead_body, 0)
            if c == 0:
                copy_w.start()
                copy_b.start()
        copy_w.wait()
        copy_b.wait()

        def switch():
            for par, u in rest:
                start_low(par, u)
            for par in range(2):
                j, r = divmod(n_low[par] * T, G)
                if r:
                    wait(in_slots(par, j).at[:, pl.ds(r, G - r), :], hsem.at[par])
                    j += 1
                wait(in_slots(par, j, n_pairs - j), hsem.at[par])
            held = []
            for c in range(SWITCH, n_steps):
                n = min(upc, n_low[c % 2] - c // 2 * upc)
                m = n - late.get(c, 0)
                slot = in_slots(c % 2, c // 2)
                if m > 0:
                    wait(slot.at[:, pl.ds(0, m * T), :], lsem.at[c])
                if n > max(m, 0):
                    held.append((slot.at[:, pl.ds(m * T, (n - m) * T), :], c))
            start_writes(0, W_FIRST)
            for view, c in held:
                wait(view, lsem.at[c])

        def step(par, j):
            g = 2 * j + par
            src = in_slots(par, j)
            dst = out_slot(par, j)

            @pl.when(g < SWITCH)
            def _():
                wait(src, lsem.at[g])

            if SWITCH % 2 == par:
                pl.when(g == SWITCH)(switch)

            bias = b_v[...].astype(jnp.float32)[None, :]
            for s in range(n_sub):
                k, r0 = s // spr, s % spr * SUB
                acc = jnp.dot(src[k, r0:r0 + SUB, :], w_v[0, 0],
                              preferred_element_type=jnp.float32)
                dst[k, r0:r0 + SUB, :] = (acc + bias).astype(dst.dtype)

                @pl.when(g < SWITCH)
                def _():
                    start_high(1 - par, j, s)

                if s in l_slots:
                    u = lead[1 - par] + j * L_STEP + l_slots.index(s)

                    @pl.when(jnp.logical_and(u < n_low[1 - par], g < SWITCH))
                    def _():
                        start_low(1 - par, u)

                if s in w_slots:
                    u = W_FIRST + (g - SWITCH) * W_STEP + w_slots.index(s)
                    start_write(jnp.maximum(u, 0), g >= SWITCH)

        def pair(j, carry):
            step(0, j)
            step(1, j)
            return carry

        lax.fori_loop(0, n_pairs, pair, 0)
        start_writes(w_in_loop, 2 * n_units)
        wait(o_hbm, wsem)

    out = pl.pallas_call(
        kernel,
        in_specs=[pl.BlockSpec(memory_space=pl.ANY)] * 3,
        out_specs=pl.BlockSpec(memory_space=pl.ANY),
        out_shape=jax.ShapeDtypeStruct((K, S, C), x.dtype),
        scratch_shapes=[
            pltpu.VMEM((n_pairs, K, G, C), x.dtype),
            pltpu.VMEM((n_pairs + 1, K, G, C), x.dtype),
            pltpu.VMEM(w.shape, w.dtype),
            pltpu.VMEM(b.shape, b.dtype),
            pltpu.SemaphoreType.DMA((n_steps,)),
            pltpu.SemaphoreType.DMA((2,)),
            pltpu.SemaphoreType.DMA((2,)),
            pltpu.SemaphoreType.DMA(()),
        ],
        compiler_params=pltpu.CompilerParams(
            vmem_limit_bytes=124 * 1024 * 1024,
            disable_bounds_checks=True,
            disable_semaphore_checks=True,
        ),
    )(x.reshape(K, S, C), w, b)
    return out.reshape(B, H, W, C)
```

```python
import jax
import jax.numpy as jnp
from jax import lax
import jax.experimental.pallas as pl
import jax.experimental.pallas.tpu as pltpu

REGION = 4096
NSTREAM = 6
CHUNK = 256
UNITS = (40, 48, 40)
SUB = 64
PIECE = 8
SWITCH = 57
LEAD = 6
L_STEP = 3
W_FIRST = 8
W_STEP = 3
EARLY = 96


def _spread(n, m):
    return [s for s in range(m) if (s * n) // m != ((s + 1) * n) // m]


@jax.jit
def pallas_standalone__standard_2d_1d_3d_conv__vision_kernel(
    x: jax.Array,
    w: jax.Array,
    b: jax.Array,
):
    B, H, W, C = x.shape
    assert w.shape == (1, 1, C, C) and b.shape == (C,)
    S, K, G, P = REGION, NSTREAM, CHUNK, sum(UNITS)
    n_regions = B * H * W // S
    cpb = S // G
    n_steps = n_regions // K * cpb
    n_pairs = n_steps // 2
    gpc = G // P
    spr = G // SUB
    n_sub = K * spr
    assert n_regions * S == B * H * W and n_regions % K == 0
    assert cpb * G == S and n_steps % 2 == 0 and gpc * P == G and spr * SUB == G
    assert G % PIECE == 0 and all(n % 8 == 0 for n in UNITS + (PIECE, EARLY))
    units = [(sum(UNITS[:i]), n) for i, n in enumerate(UNITS)]

    low_rows = [n_pairs * G - (SWITCH + p) // 2 * spr * PIECE for p in range(2)]
    low_groups = [r // P for r in low_rows]
    order = [(c % 2, c // 2 * gpc + i)
             for c in range(n_steps) for i in range(gpc)][:LEAD]
    lead = [sum(p == q for p, _ in order) for q in range(2)]
    for g in range(SWITCH):
        assert all((g % 2, g // 2 * gpc + i) in order for i in range(gpc))
        p = 1 - g % 2
        lo = lead[p] + g // 2 * L_STEP
        order += [(p, t) for t in range(lo, min(lo + L_STEP, low_groups[p]))]
    copies = [(p, t * P + o, n) for p, t in order for o, n in units]
    rest = []
    for p in (1, 0):
        rest += [(p, t * P + o, n) for t in range(low_groups[p])
                 if (p, t) not in order for o, n in units]
        rest += [(p, r, min(max(UNITS), low_rows[p] - r))
                 for r in range(low_groups[p] * P, low_rows[p], max(UNITS))]
    late, left = {}, EARLY
    for p, r, n in reversed(copies + rest):
        if left > 0:
            c = 2 * (r // G) + p
            late[c] = late.get(c, 0) + min(n, left)
            left -= n
    assert min(late) >= SWITCH
    assert W_FIRST <= SWITCH * gpc
    for g in range(SWITCH, n_steps):
        assert W_FIRST + (g - SWITCH + 1) * W_STEP <= g * gpc
    w_in_loop = W_FIRST + (n_steps - SWITCH) * W_STEP
    assert w_in_loop <= n_steps * gpc
    l_slots = _spread(L_STEP * len(units), n_sub)
    w_slots = _spread(W_STEP * len(units), n_sub)

    def kernel(x_hbm, w_hbm, b_hbm, o_hbm, buf_a, buf_b, w_v, b_v,
               lsem, hsem, psem, wsem):
        def in_slots(par, j, n=None):
            ref, j = (buf_a, j) if par == 0 else (buf_b, j + 1)
            return ref.at[j] if n is None else ref.at[pl.ds(j, n)]

        def out_slot(par, j):
            return buf_b.at[j] if par == 0 else buf_a.at[j]

        def in_hbm(c, off):
            row = pl.multiple_of(lax.rem(c, cpb) * G + off, 8)
            return lax.div(c, cpb) * K, row

        def in_vmem(row):
            return lax.div(row, G), pl.multiple_of(lax.rem(row, G), 8)

        def start_low(par, row, n):
            j, off = in_vmem(row)
            r0, hrow = in_hbm(2 * j + par, off)
            pltpu.make_async_copy(
                x_hbm.at[pl.ds(r0, K), pl.ds(hrow, n), :],
                in_slots(par, j).at[:, pl.ds(off, n), :],
                lsem.at[2 * j + par]).start(priority=1)

        def start_high(par, n, s):
            j, off = in_vmem(low_rows[par] + (n * spr + s % spr) * PIECE)
            r0, hrow = in_hbm(2 * j + par, off)
            pltpu.make_async_copy(
                x_hbm.at[r0 + s // spr, pl.ds(hrow, PIECE), :],
                in_slots(par, j).at[s // spr, pl.ds(off, PIECE), :],
                hsem.at[par]).start(priority=0)

        def start_write(t, i, enable=True):
            c = lax.div(t, gpc)
            off = pl.multiple_of(lax.rem(t, gpc) * P + units[i][0], 8)
            r0, hrow = in_hbm(c, off)
            n = units[i][1]
            for par in range(2):
                @pl.when(jnp.logical_and(lax.rem(c, 2) == par, enable))
                def _():
                    pltpu.make_async_copy(
                        out_slot(par, lax.div(c, 2)).at[:, pl.ds(off, n), :],
                        o_hbm.at[pl.ds(r0, K), pl.ds(hrow, n), :], wsem).start()

        def start_writes(lo, hi):
            def body(t, carry):
                for i in range(len(units)):
                    start_write(t, i)
                return carry
            lax.fori_loop(lo, hi, body, 0)

        def wait(view, sem):
            pltpu.make_async_copy(view, view, sem).wait()

        copy_w = pltpu.make_async_copy(w_hbm, w_v, psem.at[0])
        copy_b = pltpu.make_async_copy(b_hbm, b_v, psem.at[1])
        for i, args in enumerate(copies[:LEAD * len(units)]):
            start_low(*args)
            if i == len(units) - 1:
                copy_w.start()
                copy_b.start()
        copy_w.wait()
        copy_b.wait()

        def switch():
            for args in rest:
                start_low(*args)
            for par in range(2):
                j, r = divmod(low_rows[par], G)
                if r:
                    wait(in_slots(par, j).at[:, pl.ds(r, G - r), :], hsem.at[par])
                    j += 1
                if j < n_pairs:
                    wait(in_slots(par, j, n_pairs - j), hsem.at[par])
            held = []
            for c in range(SWITCH, n_steps):
                n = min(G, low_rows[c % 2] - c // 2 * G)
                m = n - late.get(c, 0)
                slot = in_slots(c % 2, c // 2)
                if m > 0:
                    wait(slot.at[:, pl.ds(0, m), :], lsem.at[c])
                if n > max(m, 0):
                    held.append((slot.at[:, pl.ds(m, n - m), :], lsem.at[c]))
            start_writes(0, W_FIRST)
            for view, sem in held:
                wait(view, sem)

        def step(par, j):
            g = 2 * j + par
            src = in_slots(par, j)
            dst = out_slot(par, j)

            @pl.when(g < SWITCH)
            def _():
                wait(src, lsem.at[g])

            if SWITCH % 2 == par:
                pl.when(g == SWITCH)(switch)

            bias = b_v[...].astype(jnp.float32)[None, :]
            for s in range(n_sub):
                k, r0 = s // spr, s % spr * SUB
                acc = jnp.dot(src[k, r0:r0 + SUB, :], w_v[0, 0],
                              preferred_element_type=jnp.float32)
                dst[k, r0:r0 + SUB, :] = (acc + bias).astype(dst.dtype)

                @pl.when(g < SWITCH)
                def _():
                    start_high(1 - par, j, s)

                if s in l_slots:
                    q, i = divmod(l_slots.index(s), len(units))
                    t = lead[1 - par] + j * L_STEP + q

                    @pl.when(jnp.logical_and(t < low_groups[1 - par], g < SWITCH))
                    def _():
                        start_low(1 - par, t * P + units[i][0], units[i][1])

                if s in w_slots:
                    q, i = divmod(w_slots.index(s), len(units))
                    t = W_FIRST + (g - SWITCH) * W_STEP + q
                    start_write(jnp.maximum(t, 0), i, g >= SWITCH)

        def pair(j, carry):
            step(0, j)
            step(1, j)
            return carry

        lax.fori_loop(0, n_pairs, pair, 0)
        start_writes(w_in_loop, n_steps * gpc)
        wait(o_hbm, wsem)

    out = pl.pallas_call(
        kernel,
        in_specs=[pl.BlockSpec(memory_space=pl.ANY)] * 3,
        out_specs=pl.BlockSpec(memory_space=pl.ANY),
        out_shape=jax.ShapeDtypeStruct((n_regions, S, C), x.dtype),
        scratch_shapes=[
            pltpu.VMEM((n_pairs, K, G, C), x.dtype),
            pltpu.VMEM((n_pairs + 1, K, G, C), x.dtype),
            pltpu.VMEM(w.shape, w.dtype),
            pltpu.VMEM(b.shape, b.dtype),
            pltpu.SemaphoreType.DMA((n_steps,)),
            pltpu.SemaphoreType.DMA((2,)),
            pltpu.SemaphoreType.DMA((2,)),
            pltpu.SemaphoreType.DMA(()),
        ],
        compiler_params=pltpu.CompilerParams(
            vmem_limit_bytes=124 * 1024 * 1024,
            disable_bounds_checks=True,
            disable_semaphore_checks=True,
        ),
    )(x.reshape(n_regions, S, C), w, b)
    return out.reshape(B, H, W, C)
```

```python
import jax
import jax.numpy as jnp
from jax import lax
import jax.experimental.pallas as pl
import jax.experimental.pallas.tpu as pltpu

REGION = 4096
NSTREAM = 6
CHUNK = 256
IN_UNITS = (24, 40)
OUT_UNITS = (40, 32, 40, 32, 40, 32, 40)
SUB = 64
PIECE = 8
SWITCH = 57
LEAD = 12
L_STEP = 6
W_FIRST = 4
W_STEP = (10, 11)
EARLY = 96


def _spread(n, m):
    return [s for s in range(m) if (s * n) // m != ((s + 1) * n) // m]


@jax.jit
def pallas_standalone__standard_2d_1d_3d_conv__vision_kernel(
    x: jax.Array,
    w: jax.Array,
    b: jax.Array,
):
    B, H, W, C = x.shape
    assert w.shape == (1, 1, C, C) and b.shape == (C,)
    S, K, G, P = REGION, NSTREAM, CHUNK, sum(IN_UNITS)
    n_regions = B * H * W // S
    cpb = S // G
    n_steps = n_regions // K * cpb
    n_pairs = n_steps // 2
    gpc = G // P
    spr = G // SUB
    n_sub = K * spr
    assert n_regions * S == B * H * W and n_regions % K == 0
    assert cpb * G == S and n_steps % 2 == 0 and gpc * P == G and spr * SUB == G
    assert G % PIECE == 0 and sum(OUT_UNITS) == G
    assert all(n % 8 == 0 for n in IN_UNITS + OUT_UNITS + (PIECE, EARLY))
    units = [(sum(IN_UNITS[:i]), n) for i, n in enumerate(IN_UNITS)]
    out_units = [(sum(OUT_UNITS[:i]), n) for i, n in enumerate(OUT_UNITS)]
    upc = len(out_units)

    low_rows = [n_pairs * G - (SWITCH + p) // 2 * spr * PIECE for p in range(2)]
    low_groups = [r // P for r in low_rows]
    order = [(c % 2, c // 2 * gpc + i)
             for c in range(n_steps) for i in range(gpc)][:LEAD]
    lead = [sum(p == q for p, _ in order) for q in range(2)]
    for g in range(SWITCH):
        assert all((g % 2, g // 2 * gpc + i) in order for i in range(gpc))
        p = 1 - g % 2
        lo = lead[p] + g // 2 * L_STEP
        order += [(p, t) for t in range(lo, min(lo + L_STEP, low_groups[p]))]
    copies = [(p, t * P + o, n) for p, t in order for o, n in units]
    rest = []
    for p in (1, 0):
        rest += [(p, t * P + o, n) for t in range(low_groups[p])
                 if (p, t) not in order for o, n in units]
        rest += [(p, r, min(max(IN_UNITS), low_rows[p] - r))
                 for r in range(low_groups[p] * P, low_rows[p], max(IN_UNITS))]
    late, left = {}, EARLY
    for p, r, n in reversed(copies + rest):
        if left > 0:
            c = 2 * (r // G) + p
            late[c] = late.get(c, 0) + min(n, left)
            left -= n
    assert min(late) >= SWITCH
    assert W_FIRST <= SWITCH and sum(W_STEP) % upc == 0
    w_in_loop = W_FIRST * upc
    for g in range(SWITCH, n_steps):
        w_in_loop += W_STEP[(g - SWITCH) % 2]
        assert w_in_loop <= g * upc
    l_slots = _spread(L_STEP * len(units), n_sub)
    w_slots = [_spread(n, n_sub) for n in W_STEP]

    def kernel(x_hbm, w_hbm, b_hbm, o_hbm, buf_a, buf_b, w_v, b_v,
               lsem, hsem, psem, wsem):
        def in_slots(par, j, n=None):
            ref, j = (buf_a, j) if par == 0 else (buf_b, j + 1)
            return ref.at[j] if n is None else ref.at[pl.ds(j, n)]

        def out_slot(par, j):
            return buf_b.at[j] if par == 0 else buf_a.at[j]

        def in_hbm(c, off):
            row = pl.multiple_of(lax.rem(c, cpb) * G + off, 8)
            return lax.div(c, cpb) * K, row

        def in_vmem(row):
            return lax.div(row, G), pl.multiple_of(lax.rem(row, G), 8)

        def start_low(par, row, n):
            j, off = in_vmem(row)
            r0, hrow = in_hbm(2 * j + par, off)
            pltpu.make_async_copy(
                x_hbm.at[pl.ds(r0, K), pl.ds(hrow, n), :],
                in_slots(par, j).at[:, pl.ds(off, n), :],
                lsem.at[2 * j + par]).start(priority=1)

        def start_high(par, n, s):
            j, off = in_vmem(low_rows[par] + (n * spr + s % spr) * PIECE)
            r0, hrow = in_hbm(2 * j + par, off)
            pltpu.make_async_copy(
                x_hbm.at[r0 + s // spr, pl.ds(hrow, PIECE), :],
                in_slots(par, j).at[s // spr, pl.ds(off, PIECE), :],
                hsem.at[par]).start(priority=0)

        def start_write(c, i, enable=True):
            off, n = out_units[i]
            r0, hrow = in_hbm(c, off)
            for par in range(2):
                @pl.when(jnp.logical_and(lax.rem(c, 2) == par, enable))
                def _():
                    pltpu.make_async_copy(
                        out_slot(par, lax.div(c, 2)).at[:, pl.ds(off, n), :],
                        o_hbm.at[pl.ds(r0, K), pl.ds(hrow, n), :], wsem).start()

        def start_writes(lo, hi):
            def body(c, carry):
                for i in range(upc):
                    start_write(c, i)
                return carry
            lax.fori_loop(lo, hi, body, 0)

        def wait(view, sem):
            pltpu.make_async_copy(view, view, sem).wait()

        copy_w = pltpu.make_async_copy(w_hbm, w_v, psem.at[0])
        copy_b = pltpu.make_async_copy(b_hbm, b_v, psem.at[1])
        for i, args in enumerate(copies[:LEAD * len(units)]):
            start_low(*args)
            if i == len(units) - 1:
                copy_w.start()
                copy_b.start()
        copy_w.wait()
        copy_b.wait()

        def switch():
            for args in rest:
                start_low(*args)
            for par in range(2):
                j, r = divmod(low_rows[par], G)
                if r:
                    wait(in_slots(par, j).at[:, pl.ds(r, G - r), :], hsem.at[par])
                    j += 1
                if j < n_pairs:
                    wait(in_slots(par, j, n_pairs - j), hsem.at[par])
            held = []
            for c in range(SWITCH, n_steps):
                n = min(G, low_rows[c % 2] - c // 2 * G)
                m = n - late.get(c, 0)
                slot = in_slots(c % 2, c // 2)
                if m > 0:
                    wait(slot.at[:, pl.ds(0, m), :], lsem.at[c])
                if n > max(m, 0):
                    held.append((slot.at[:, pl.ds(m, n - m), :], lsem.at[c]))
            start_writes(0, W_FIRST)
            for view, sem in held:
                wait(view, sem)

        def step(par, j):
            g = 2 * j + par
            src = in_slots(par, j)
            dst = out_slot(par, j)

            @pl.when(g < SWITCH)
            def _():
                wait(src, lsem.at[g])

            if SWITCH % 2 == par:
                pl.when(g == SWITCH)(switch)

            bias = b_v[...].astype(jnp.float32)[None, :]
            for s in range(n_sub):
                k, r0 = s // spr, s % spr * SUB
                acc = jnp.dot(src[k, r0:r0 + SUB, :], w_v[0, 0],
                              preferred_element_type=jnp.float32)
                dst[k, r0:r0 + SUB, :] = (acc + bias).astype(dst.dtype)

                @pl.when(g < SWITCH)
                def _():
                    start_high(1 - par, j, s)

                if s in l_slots:
                    q, i = divmod(l_slots.index(s), len(units))
                    t = lead[1 - par] + j * L_STEP + q

                    @pl.when(jnp.logical_and(t < low_groups[1 - par], g < SWITCH))
                    def _():
                        start_low(1 - par, t * P + units[i][0], units[i][1])

                odd = (par - SWITCH) % 2
                if s in w_slots[odd]:
                    q, i = divmod(odd * W_STEP[0] + w_slots[odd].index(s), upc)
                    pairs = lax.div(jnp.maximum(g - SWITCH, 0), 2)
                    c = W_FIRST + pairs * (sum(W_STEP) // upc) + q
                    start_write(c, i, g >= SWITCH)

        def pair(j, carry):
            step(0, j)
            step(1, j)
            return carry

        lax.fori_loop(0, n_pairs, pair, 0)
        for i in range(w_in_loop % upc, upc if w_in_loop % upc else 0):
            start_write(w_in_loop // upc, i)
        start_writes(-(-w_in_loop // upc), n_steps)
        wait(o_hbm, wsem)

    out = pl.pallas_call(
        kernel,
        in_specs=[pl.BlockSpec(memory_space=pl.ANY)] * 3,
        out_specs=pl.BlockSpec(memory_space=pl.ANY),
        out_shape=jax.ShapeDtypeStruct((n_regions, S, C), x.dtype),
        scratch_shapes=[
            pltpu.VMEM((n_pairs, K, G, C), x.dtype),
            pltpu.VMEM((n_pairs + 1, K, G, C), x.dtype),
            pltpu.VMEM(w.shape, w.dtype),
            pltpu.VMEM(b.shape, b.dtype),
            pltpu.SemaphoreType.DMA((n_steps,)),
            pltpu.SemaphoreType.DMA((2,)),
            pltpu.SemaphoreType.DMA((2,)),
            pltpu.SemaphoreType.DMA(()),
        ],
        compiler_params=pltpu.CompilerParams(
            vmem_limit_bytes=124 * 1024 * 1024,
            disable_bounds_checks=True,
            disable_semaphore_checks=True,
        ),
    )(x.reshape(n_regions, S, C), w, b)
    return out.reshape(B, H, W, C)
```

```python
import jax
import jax.numpy as jnp
from jax import lax
import jax.experimental.pallas as pl
import jax.experimental.pallas.tpu as pltpu

REGION = 4096
NSTREAM = 6
CHUNK = 256
IN_UNITS = (32, 48, 40, 40, 48, 48)
OUT_UNITS = (40, 40, 48, 40, 40, 48)
SUB = 64
PIECE = 8
SWITCH = 57
LEAD = 3
L_STEP = (2, 1)
EARLY = 576
W_FIRST = 4
W_STEP = (9, 9)


def _spread(n, m):
    return [s for s in range(m) if (s * n) // m != ((s + 1) * n) // m]


def _offsets(sizes):
    return [(sum(sizes[:i]), n) for i, n in enumerate(sizes)]


@jax.jit
def pallas_standalone__standard_2d_1d_3d_conv__vision_kernel(
    x: jax.Array,
    w: jax.Array,
    b: jax.Array,
):
    B, H, W, C = x.shape
    assert w.shape == (1, 1, C, C) and b.shape == (C,)
    S, K, G = REGION, NSTREAM, CHUNK
    n_regions = B * H * W // S
    cpb = S // G
    n_steps = n_regions // K * cpb
    n_pairs = n_steps // 2
    spr = G // SUB
    n_sub = K * spr
    ppr = G // PIECE
    ppc = K * ppr
    in_units, out_units = _offsets(IN_UNITS), _offsets(OUT_UNITS)
    upc = len(out_units)
    assert n_regions * S == B * H * W and n_regions % K == 0 and cpb * G == S
    assert n_steps % 2 == 0 and spr * SUB == G and ppr * PIECE == G
    assert sum(IN_UNITS) == G and sum(OUT_UNITS) == G
    assert all(n % 8 == 0 for n in IN_UNITS + OUT_UNITS + (PIECE,))

    first = [n_pairs * ppc - (SWITCH + p) // 2 * n_sub for p in range(2)]
    whole = [u // ppc for u in first]
    lead = [(LEAD + 1) // 2, LEAD // 2]
    asked = list(lead)
    for g in range(SWITCH):
        assert g // 2 < asked[g % 2]
        p = 1 - g % 2
        asked[p] = min(asked[p] + L_STEP[g // 2 % 2], whole[p])
    rest = []
    for p in (1, 0):
        for j in range(asked[p], whole[p]):
            rest += [(p, j, 0, K, off, n) for off, n in in_units]
        k, r = divmod(first[p] % ppc, ppr)
        rest += [(p, whole[p], k, 1, 0, r * PIECE)] if r else []
        rest += [(p, whole[p], 0, k, off, n) for off, n in in_units] if k else []
    n_wait, left = len(rest), EARLY
    while left > 0:
        n_wait -= 1
        left -= rest[n_wait][3] * rest[n_wait][5]
    assert n_wait >= 0
    assert W_FIRST <= SWITCH and sum(W_STEP) % upc == 0
    w_in_loop = W_FIRST * upc
    for g in range(SWITCH, n_steps):
        w_in_loop += W_STEP[(g - SWITCH) % 2]
        assert w_in_loop <= g * upc
    l_slots = _spread(max(L_STEP) * len(in_units), n_sub)
    w_slots = [_spread(n, n_sub) for n in W_STEP]

    def kernel(x_hbm, w_hbm, b_hbm, o_hbm, buf_a, buf_b, w_v, b_v,
               lsem, hsem, psem, wsem):
        def in_slots(par, j, n=None):
            ref, j = (buf_a, j) if par == 0 else (buf_b, j + 1)
            return ref.at[j] if n is None else ref.at[pl.ds(j, n)]

        def out_slot(par, j):
            return buf_b.at[j] if par == 0 else buf_a.at[j]

        def in_hbm(c, off):
            row = pl.multiple_of(lax.rem(c, cpb) * G + off, 8)
            return lax.div(c, cpb) * K, row

        def low_copy(par, j, k, nk, off, n):
            r0, row = in_hbm(2 * j + par, off)
            return pltpu.make_async_copy(
                x_hbm.at[pl.ds(r0 + k, nk), pl.ds(row, n), :],
                in_slots(par, j).at[pl.ds(k, nk), pl.ds(off, n), :],
                lsem.at[2 * j + par])

        def start_high(par, q):
            u = first[par] + q
            j = lax.div(u, ppc)
            k = lax.div(lax.rem(u, ppc), ppr)
            off = pl.multiple_of(lax.rem(u, ppr) * PIECE, 8)
            r0, row = in_hbm(2 * j + par, off)
            pltpu.make_async_copy(
                x_hbm.at[r0 + k, pl.ds(row, PIECE), :],
                in_slots(par, j).at[k, pl.ds(off, PIECE), :],
                hsem.at[par]).start(priority=0)

        def start_write(c, i, enable=True):
            off, n = out_units[i]
            r0, row = in_hbm(c, off)
            for par in range(2):
                @pl.when(jnp.logical_and(lax.rem(c, 2) == par, enable))
                def _():
                    pltpu.make_async_copy(
                        out_slot(par, lax.div(c, 2)).at[:, pl.ds(off, n), :],
                        o_hbm.at[pl.ds(r0, K), pl.ds(row, n), :], wsem).start()

        def start_writes(lo, hi):
            def body(c, carry):
                for i in range(upc):
                    start_write(c, i)
                return carry
            lax.fori_loop(lo, hi, body, 0)

        def wait(view, sem):
            pltpu.make_async_copy(view, view, sem).wait()

        copy_w = pltpu.make_async_copy(w_hbm, w_v, psem.at[0])
        copy_b = pltpu.make_async_copy(b_hbm, b_v, psem.at[1])
        for c in range(LEAD):
            for i, unit in enumerate(in_units):
                low_copy(c % 2, c // 2, 0, K, *unit).start(priority=1)
                if c == 0 and i == 1:
                    copy_w.start()
                    copy_b.start()
        copy_w.wait()
        copy_b.wait()

        def switch():
            for args in rest:
                low_copy(*args).start(priority=1)
            for par in range(2):
                j = whole[par]
                k, r = divmod(first[par] % ppc, ppr)
                if r:
                    rows = pl.ds(r * PIECE, G - r * PIECE)
                    wait(in_slots(par, j).at[k, rows, :], hsem.at[par])
                    k += 1
                if 0 < k < K:
                    wait(in_slots(par, j).at[pl.ds(k, K - k)], hsem.at[par])
                j += 1 if k else 0
                if j < n_pairs:
                    wait(in_slots(par, j, n_pairs - j), hsem.at[par])
            for c in range(SWITCH, n_steps):
                if c // 2 < asked[c % 2]:
                    wait(in_slots(c % 2, c // 2), lsem.at[c])
            for args in rest[:n_wait]:
                low_copy(*args).wait()
            start_writes(0, W_FIRST)
            for args in rest[n_wait:]:
                low_copy(*args).wait()

        def step(par, j):
            g = 2 * j + par
            src = in_slots(par, j)
            dst = out_slot(par, j)

            @pl.when(g < SWITCH)
            def _():
                wait(src, lsem.at[g])

            if SWITCH % 2 == par:
                pl.when(g == SWITCH)(switch)

            j_odd = lax.rem(j, 2)
            l_base = lead[1 - par] + lax.div(j, 2) * sum(L_STEP) + j_odd * L_STEP[0]
            w_odd = (par - SWITCH) % 2
            w_base = W_FIRST + (lax.div(jnp.maximum(g - SWITCH, 0), 2)
                                * (sum(W_STEP) // upc))
            bias = b_v[...].astype(jnp.float32)[None, :]
            for s in range(n_sub):
                k, r0 = s // spr, s % spr * SUB
                acc = jnp.dot(src[k, r0:r0 + SUB, :], w_v[0, 0],
                              preferred_element_type=jnp.float32)
                dst[k, r0:r0 + SUB, :] = (acc + bias).astype(dst.dtype)

                @pl.when(g < SWITCH)
                def _():
                    start_high(1 - par, j * n_sub + s)

                if s in l_slots:
                    q, i = divmod(l_slots.index(s), len(in_units))
                    on = jnp.logical_and(l_base + q < whole[1 - par], g < SWITCH)
                    if q >= min(L_STEP):
                        on = jnp.logical_and(on, j_odd == L_STEP.index(max(L_STEP)))

                    @pl.when(on)
                    def _():
                        low_copy(1 - par, l_base + q, 0, K,
                                 *in_units[i]).start(priority=1)

                if s in w_slots[w_odd]:
                    q, i = divmod(w_odd * W_STEP[0] + w_slots[w_odd].index(s), upc)
                    start_write(w_base + q, i, g >= SWITCH)

        def pair(j, carry):
            step(0, j)
            step(1, j)
            return carry

        lax.fori_loop(0, n_pairs, pair, 0)
        for i in range(w_in_loop % upc, upc if w_in_loop % upc else 0):
            start_write(w_in_loop // upc, i)
        start_writes(-(-w_in_loop // upc), n_steps)
        wait(o_hbm, wsem)

    out = pl.pallas_call(
        kernel,
        in_specs=[pl.BlockSpec(memory_space=pl.ANY)] * 3,
        out_specs=pl.BlockSpec(memory_space=pl.ANY),
        out_shape=jax.ShapeDtypeStruct((n_regions, S, C), x.dtype),
        scratch_shapes=[
            pltpu.VMEM((n_pairs, K, G, C), x.dtype),
            pltpu.VMEM((n_pairs + 1, K, G, C), x.dtype),
            pltpu.VMEM(w.shape, w.dtype),
            pltpu.VMEM(b.shape, b.dtype),
            pltpu.SemaphoreType.DMA((n_steps,)),
            pltpu.SemaphoreType.DMA((2,)),
            pltpu.SemaphoreType.DMA((2,)),
            pltpu.SemaphoreType.DMA(()),
        ],
        compiler_params=pltpu.CompilerParams(
            vmem_limit_bytes=124 * 1024 * 1024,
            disable_bounds_checks=True,
            disable_semaphore_checks=True,
        ),
    )(x.reshape(n_regions, S, C), w, b)
    return out.reshape(B, H, W, C)
```
